```python
import jax
import jax.numpy as jnp

def _softmax(x, axis=-1):
    return jax.nn.softmax(x, axis=axis)
def _gelu(x):
    return jax.nn.gelu(x, approximate=True)
def _silu(x):
    return jax.nn.silu(x)
def _sigmoid(x):
    return jax.nn.sigmoid(x)
def _layernorm(x, axis=-1, eps=1e-5):
    m = jnp.mean(x, axis=axis, keepdims=True)
    v = jnp.var(x, axis=axis, keepdims=True)
    return (x - m) / jnp.sqrt(v + eps)
def _scatter_add(tgt, idx, src, axis=0):
    return tgt.at[idx].add(src)
def _segment_sum(src, seg, n):
    return jax.ops.segment_sum(src, seg, n)
class _Rng:
    def __init__(self, key):
        self._k = key
    def _next(self):
        self._k, sub = jax.random.split(self._k)
        return sub
    def normal(self, shape):
        return jax.random.normal(self._next(), shape, dtype=jnp.bfloat16)
    def randint(self, lo, hi, shape):
        return jax.random.randint(self._next(), shape, lo, hi, dtype=jnp.int32)
    def uniform(self, shape, lo=0.0, hi=1.0):
        return jax.random.uniform(self._next(), shape, jnp.bfloat16, lo, hi)
    def permutation(self, n):
        return jax.random.permutation(self._next(), n)


kernel_name = 'concat_heads__ssm_conv_h3__linear_attn_block__prompt'

def setup_inputs():
    _rng = _Rng(jax.random.key(int.from_bytes(__import__("os").urandom(4), "little")))
    _w = (lambda a: (lambda t: t.astype(jnp.bfloat16) if jnp.issubdtype(t.dtype, jnp.floating) else t)(jnp.asarray(a)))
    def _A_setup():
        B, S, D = 1, 2048, 1024
        ks = 4
        return {
            "q": _w((lambda *s: _rng.normal(s) * 0.05)(B, S, D)),
            "k": _w((lambda *s: _rng.normal(s) * 0.05)(B, S, D)),
            "v": _w((lambda *s: _rng.normal(s) * 0.05)(B, S, D)),
            "shift_k": _w((lambda *s: _rng.normal(s) * 0.05)(D, ks) * 0.5),
            "ssm_k": _w((lambda *s: _rng.normal(s) * 0.05)(D, S) * (1.0 / S ** 0.5)),
            "ssm_D": _w((lambda *s: _rng.normal(s) * 0.05)(D)),
        }
    _A_in = _A_setup()

    def _B_setup():
        B, S, D = 1, 2048, 1024
        return {
            "x": _w((lambda *s: _rng.normal(s) * 0.05)(B, S, D)),
            "wqkv": _w((lambda *s: _rng.normal(s) * 0.05)(D, 3 * D)),
            "wo": _w((lambda *s: _rng.normal(s) * 0.05)(D, D)),
        }
    _B_in = _B_setup()

    return {
        "A_q": _A_in["q"],
        "A_k": _A_in["k"],
        "A_v": _A_in["v"],
        "A_shift_k": _A_in["shift_k"],
        "A_ssm_k": _A_in["ssm_k"],
        "A_ssm_D": _A_in["ssm_D"],
        "B_x": _B_in["x"],
        "B_wqkv": _B_in["wqkv"],
        "B_wo": _B_in["wo"],
    }

def reference(A_q, A_k, A_v, A_shift_k, A_ssm_k, A_ssm_D, B_x, B_wqkv, B_wo):
    def _A_ref(q, k, v, shift_k, ssm_k, ssm_D):
        B, S, D = q.shape
        ks = shift_k.shape[-1]
        k_pad = jnp.pad(k, ((0, 0), (ks - 1, 0), (0, 0)))
        k_shift = jnp.zeros_like(k)
        for t in range(ks):
            k_shift = k_shift + k_pad[:, t:t + S, :] * shift_k[:, ks - 1 - t][None, None, :]
        kv = k_shift * v
        L = 2 * S
        kv_pad = jnp.pad(kv, ((0, 0), (0, S), (0, 0)))
        kf_pad = jnp.pad(ssm_k, ((0, 0), (0, S)))
        kv_f = (lambda x, axes=(-2,-1): jnp.fft.rfft2(x.astype(jnp.float32), axes=axes))(kv_pad[:, None, :, :], axes=(1, 2))
        kf_f = (lambda x, axes=(-2,-1): jnp.fft.rfft2(x.astype(jnp.float32), axes=axes))(kf_pad[:, None, :], axes=(1, 2))
        kf_f = (lambda x, *d: x.transpose(*d))(kf_f, 1, 2, 0)
        y_f = kv_f * kf_f[None, :, :, :]
        y = (lambda x, s, axes=(-2,-1): jnp.fft.irfft2(x, s=s, axes=axes).astype(jnp.bfloat16))(y_f, (1, L), axes=(1, 2))[:, 0, :S, :]
        y = y + kv * ssm_D[None, None, :]
        return q * y

    def _B_ref(x, wqkv, wo):
        B, S, D = x.shape
        H = 32; Dh = D // H
        qkv = (lambda x, *d: x.transpose(*d))((x @ wqkv).reshape(B, S, 3, H, Dh), 2, 0, 3, 1, 4)
        q, k, v = qkv[0], qkv[1], qkv[2]
        phi = lambda t: jnp.where(t > 0, t + 1, jnp.exp(t)) + 1e-6
        pq, pk = phi(q), phi(k)
        kv = jnp.einsum("bhsd,bhse->bhde", pk, v)
        z = jnp.einsum("bhsd->bhd", pk)
        num = jnp.einsum("bhqd,bhde->bhqe", pq, kv)
        den = jnp.einsum("bhqd,bhd->bhq", pq, z)[..., None] + 1e-6
        o = num / den
        return (lambda x, *d: x.transpose(*d))(o, 0, 2, 1, 3).reshape(B, S, D) @ wo

    a = _A_ref(A_q, A_k, A_v, A_shift_k, A_ssm_k, A_ssm_D)
    b = _B_ref(B_x, B_wqkv, B_wo)
    return jnp.concatenate([a, b], axis=-1)
```

```python
import numpy as np
import ml_dtypes
import jax
import jax.numpy as jnp
import jax.experimental.pallas as pl
import jax.experimental.pallas.tpu as pltpu

S, D, C, NCH, NG = 2048, 1024, 128, 16, 8
R = 512
BF, F32, U32 = jnp.bfloat16, jnp.float32, jnp.uint32


def _dft_consts():
    fs = np.concatenate([np.arange(0, 128, 2), np.arange(1, 128, 2)]).reshape(16, 8)
    w = 2 * np.pi * (fs + 0.5) / 256.0
    t = np.arange(128)
    ang = w[:, :, None] * t[None, None, :]
    F = np.concatenate([np.cos(ang), -np.sin(ang)], axis=1).reshape(256, 128)
    G = (F / 128.0).T
    I = np.eye(128)
    b = ml_dtypes.bfloat16
    return F.astype(b), np.ascontiguousarray(G).astype(b), I.astype(b)


_F, _G, _I = _dft_consts()


class P:
    def __init__(self, ref):
        self.r = ref

    def get(self, r0, n, c0, m):
        return pltpu.bitcast(self.r[r0 // 2:(r0 + n) // 2, c0:c0 + m], BF)

    def set(self, r0, c0, val):
        n, m = val.shape
        self.r[r0 // 2:(r0 + n) // 2, c0:c0 + m] = pltpu.bitcast(val, U32)


def _nn(a, b):
    return jnp.dot(a, b, preferred_element_type=F32)


def _nt(a, b):
    return jax.lax.dot_general(a, b, (((1,), (1,)), ((), ())), preferred_element_type=F32)


def _phi(t):
    return jnp.where(t > 0, t + 1.0, jnp.exp(t)) + 1e-6


def _merge(streams):
    streams = [s for s in streams if s]
    tot = [float(sum(c for _, c in s)) for s in streams]
    pos = [0] * len(streams)
    done = [0.0] * len(streams)
    while True:
        best = None
        for i, s in enumerate(streams):
            if pos[i] < len(s):
                key = (done[i] + 0.5 * s[pos[i]][1]) / tot[i]
                if best is None or key < best[0]:
                    best = (key, i)
        if best is None:
            return
        i = best[1]
        th, c = streams[i][pos[i]]
        th()
        done[i] += c
        pos[i] += 1


def _kernel(q_h, k_h, v_h, sh_ref, sk_h, sd_ref, x_h, wqkv_h, wo_h, F_ref, G_ref, I_ref, o_h,
            q_s, k_s, v_s, sk_s, x_s, w_s, wo_s, xp, wkT, wqp, Fp, Gp, par, kf, kvp, Xs, Ks, Yp,
            pkT, Gacc, zacc, Zp, Mp, pqp, op, oA, oB, sA, sB, sW, sO):
    Fp, Gp, wkT, wqp, kvp, Yp, pkT, Zp, Mp, pqp, op = map(
        P, (Fp, Gp, wkT, wqp, kvp, Yp, pkT, Zp, Mp, pqp, op))

    def a_copies(g):
        return [pltpu.make_async_copy(k_h.at[0, :, pl.ds(g * 128, 128)], k_s.at[g], sA.at[0, g]),
                pltpu.make_async_copy(v_h.at[0, :, pl.ds(g * 128, 128)], v_s.at[g], sA.at[1, g]),
                pltpu.make_async_copy(sk_h.at[pl.ds(g * 128, 128), :], sk_s.at[g], sA.at[2, g]),
                pltpu.make_async_copy(q_h.at[0, :, pl.ds(g * 128, 128)], q_s.at[g], sA.at[3, g])]

    def x_copy(i):
        return pltpu.make_async_copy(x_h.at[0, pl.ds(i * R, R), :], x_s.at[i], sB.at[i])

    def w_copy(j):
        return pltpu.make_async_copy(wqkv_h.at[:, pl.ds(j * D, D)], w_s.at[j], sW.at[j])

    wo_copy = pltpu.make_async_copy(wo_h, wo_s, sW.at[3])

    def oa_copy(g):
        return pltpu.make_async_copy(oA.at[g], o_h.at[0, :, pl.ds(g * 128, 128)], sO.at[0, g])

    def ob_copy(i):
        return pltpu.make_async_copy(oB.at[i], o_h.at[0, pl.ds(i * R, R), pl.ds(D, D)], sO.at[1, i])

    w_copy(1).start()
    x_copy(0).start()
    for c in a_copies(0):
        c.start()
    for i in range(1, 4):
        x_copy(i).start()
        for c in a_copies(i):
            c.start()
    w_copy(2).start()
    wo_copy.start()
    w_copy(0).start()
    for g in range(4, NG):
        for c in a_copies(g):
            c.start()

    Fp.set(0, 0, F_ref[...])
    Gp.set(0, 0, G_ref[...])
    shT = sh_ref[...].astype(F32).T
    sd = sd_ref[...].astype(F32)
    for g in range(NG):
        par[g, 0:4, :] = shT[:, g * 128:(g + 1) * 128]
        par[g, 4:5, :] = sd[:, g * 128:(g + 1) * 128]
    kf[0:8, :] = jnp.zeros((8, 128), F32)
    zacc[...] = jnp.zeros(zacc.shape, F32)
    Gacc[...] = jnp.zeros(Gacc.shape, F32)
    w_copy(1).wait()
    eye = I_ref[...]
    for a in range(8):
        for b in range(8):
            t = _nt(eye, w_s[1, a * 128:(a + 1) * 128, b * 128:(b + 1) * 128])
            wkT.set(b * 128, a * 128, t.astype(BF))

    def a_shift(g):
        out = []
        for r in range(0, S, 128):
            def th(r=r):
                kf[8 + r:8 + r + 128, :] = k_s[g, r:r + 128, :].astype(F32)
            out.append((th, 16))
        for r in range(0, S, 32):
            def th(r=r):
                acc = kf[8 + r:8 + r + 32, :] * par[g, 0:1, :]
                for i in range(1, 4):
                    acc = acc + kf[8 + r - i:8 + r - i + 32, :] * par[g, i:i + 1, :]
                kvp.set(r, 0, (acc * v_s[g, r:r + 32, :].astype(F32)).astype(BF))
            out.append((th, 40))
        return out

    def a_dft(g):
        out = []
        for n in range(NCH):
            def th(n=n):
                Ks[n * 256:(n + 1) * 256, :] = _nt(Fp.get(0, 256, 0, 128), sk_s[g, :, n * 128:(n + 1) * 128])
            out.append((th, 64))
        for n in range(NCH):
            def th(n=n):
                Xs[n * 256:(n + 1) * 256, :] = _nn(Fp.get(0, 256, 0, 128), kvp.get(n * 128, 128, 0, 128))
            out.append((th, 64))
        return out

    def a_conv():
        out = []
        for fg in range(16):
            def ld(ref, n, p, fg=fg):
                o = n * 256 + 16 * fg + 8 * p
                return ref[o:o + 8, :]

            def thk(fg=fg, ld=ld):
                for m in range(NCH - 1, 0, -1):
                    kr, ki = ld(Ks, m, 0), ld(Ks, m, 1)
                    pr, pi = ld(Ks, m - 1, 0), ld(Ks, m - 1, 1)
                    o = m * 256 + 16 * fg
                    if fg < 8:
                        Ks[o:o + 8, :] = kr - pi
                        Ks[o + 8:o + 16, :] = ki + pr
                    else:
                        Ks[o:o + 8, :] = kr + pi
                        Ks[o + 8:o + 16, :] = ki - pr
            out.append((thk, 30))
            for n in range(NCH):
                def th(n=n, fg=fg, ld=ld):
                    ar = ai = None
                    for m in range(n + 1):
                        kr, ki = ld(Ks, m, 0), ld(Ks, m, 1)
                        xr, xi = ld(Xs, n - m, 0), ld(Xs, n - m, 1)
                        tr = kr * xr - ki * xi
                        ti = kr * xi + ki * xr
                        ar = tr if ar is None else ar + tr
                        ai = ti if ai is None else ai + ti
                    Yp.set(n * 256 + 16 * fg, 0, jnp.concatenate([ar, ai], axis=0).astype(BF))
                out.append((th, 8 * (n + 1)))
        return out

    def a_inv(g):
        out = []
        for n in range(NCH):
            def th(n=n):
                y = _nn(Gp.get(0, 128, 0, 256), Yp.get(n * 256, 256, 0, 128))
                kv = kvp.get(n * 128, 128, 0, 128).astype(F32)
                y = y + kv * par[g, 4:5, :]
                oA[g, n * 128:(n + 1) * 128, :] = (q_s[g, n * 128:(n + 1) * 128, :].astype(F32) * y).astype(BF)
            out.append((th, 64))
        return out

    def run_step(g, b):
        n = len(b)
        n1, n3 = n // 8, n - n // 8
        for c in a_copies(g):
            c.wait()
        _merge([b[:n1], a_shift(g)])
        _merge([a_dft(g)])
        _merge([b[n1:n3], a_conv()])
        _merge([b[n3:], a_inv(g)])
        oa_copy(g).start()

    def b1(i):
        X = P(xp.at[i])

        def kproj(c):
            out = []
            for t in range(R // 128):
                st = {}
                for kh in range(2):
                    def th(t=t, kh=kh, st=st):
                        r = _nt(wkT.get(c * 64, 64, kh * 512, 512), X.get(t * 128, 128, kh * 512, 512))
                        if kh == 0:
                            st["a"] = r
                            return
                        p = _phi(r + st["a"])
                        zacc[c * 64:(c + 1) * 64, :] += p
                        pkT.set(c * 64, t * 128, p.astype(BF))
                    out.append((th, 64))
            return out

        def gup(c):
            out = []
            for h in range(8):
                def th(h=h):
                    Gacc[c * 64:(c + 1) * 64, h * 128:(h + 1) * 128] += _nn(
                        pkT.get(c * 64, 64, 0, R), X.get(0, R, h * 128, 128))
                out.append((th, 64))
            return out

        seq = kproj(0)
        for c in range(1, 16):
            seq += kproj(c) + gup(c - 1)
        return seq + gup(15)

    def step1(i, carry):
        x_copy(i).wait()
        for r in range(0, R, 64):
            P(xp.at[i]).set(r, 0, x_s[i, r:r + 64, :])
        run_step(i, b1(i))
        return carry

    jax.lax.fori_loop(0, 4, step1, 0)

    w_copy(2).wait()
    wo_copy.wait()
    w_copy(0).wait()
    for r in range(0, D, 64):
        wqp.set(r, 0, w_s[0, r:r + 64, :])
    ri = jax.lax.broadcasted_iota(jnp.int32, (128, 128), 0) // 32
    ci = jax.lax.broadcasted_iota(jnp.int32, (128, 128), 1) // 32
    mask = ri == ci
    kvs = []
    for g in range(NG):
        z = jnp.sum(zacc[g * 128:(g + 1) * 128, :], axis=1, keepdims=True)
        Zp.set(g * 128, 0, jnp.where(mask, z, 0.0).astype(BF))
        kv = _nn(Gacc[g * 128:(g + 1) * 128, :].astype(BF), w_s[2, :, g * 128:(g + 1) * 128])
        kvs.append(jnp.where(mask, kv, 0.0).astype(BF))
    for g in range(NG):
        for h in range(2):
            Mp.set(g * 128, h * 512, _nn(kvs[g], wo_s[g * 128:(g + 1) * 128, h * 512:(h + 1) * 512]).astype(BF))

    def b2(i):
        X = P(xp.at[i])

        def qproj(t):
            out = []
            for h in range(8):
                st = {}
                for kh in range(2):
                    def th(h=h, kh=kh, st=st):
                        r = _nn(X.get(t * 64, 64, kh * 512, 512), wqp.get(kh * 512, 512, h * 128, 128))
                        if kh == 0:
                            st["a"] = r
                            return
                        pqp.set((t % 2) * 64, h * 128, _phi(r + st["a"]).astype(BF))
                    out.append((th, 64))
            return out

        def den(t):
            out = []
            for hh in range(2):
                def th(hh=hh):
                    for h in range(hh * 4, hh * 4 + 4):
                        pq = pqp.get((t % 2) * 64, 64, h * 128, 128)
                        d = _nn(pq, Zp.get(h * 128, 128, 0, 128)) + 1e-6
                        op.set((t % 2) * 64, h * 128, (pq.astype(F32) / d).astype(BF))
                out.append((th, 64))
            return out

        def oproj(t):
            out = []
            for h in range(8):
                st = {}
                for kh in range(2):
                    def th(h=h, kh=kh, st=st):
                        r = _nn(op.get((t % 2) * 64, 64, kh * 512, 512), Mp.get(kh * 512, 512, h * 128, 128))
                        if kh == 0:
                            st["a"] = r
                            return
                        oB[i, t * 64:(t + 1) * 64, h * 128:(h + 1) * 128] = (r + st["a"]).astype(BF)
                    out.append((th, 64))
            return out

        nt = R // 64
        seq = qproj(0)
        for t in range(nt):
            if t + 1 < nt:
                nx = qproj(t + 1)
                seq += nx[:2] + den(t) + nx[2:]
            else:
                seq += den(t)
            seq += oproj(t)
        return seq

    def step2(i, carry):
        run_step(i + 4, b2(i))
        ob_copy(i).start()
        return carry

    jax.lax.fori_loop(0, 4, step2, 0)

    for g in range(NG):
        oa_copy(g).wait()
    for i in range(4):
        ob_copy(i).wait()


@jax.jit
def pallas_concat_heads__ssm_conv_h3__linear_attn_block__prompt_kernel(
    A_q, A_k, A_v, A_shift_k, A_ssm_k, A_ssm_D, B_x, B_wqkv, B_wo,
):
    anyspec = pl.BlockSpec(memory_space=pl.ANY)
    vm = pl.BlockSpec(memory_space=pltpu.VMEM)
    V = pltpu.VMEM
    scratch = [
        V((NG, S, 128), BF), V((NG, S, 128), BF), V((NG, S, 128), BF), V((NG, 128, S), BF),
        V((4, R, D), BF), V((3, D, D), BF), V((D, D), BF),
        V((4, R // 2, D), U32), V((D // 2, D), U32), V((D // 2, D), U32),
        V((128, 128), U32), V((64, 256), U32), V((NG, 8, 128), F32), V((S + 8, 128), F32),
        V((S // 2, 128), U32), V((2 * S, 128), F32), V((2 * S, 128), F32), V((S, 128), U32),
        V((D // 2, R), U32), V((D, D), F32), V((D, 128), F32), V((D // 2, 128), U32),
        V((D // 2, D), U32), V((64, D), U32), V((64, D), U32),
        V((NG, S, 128), BF), V((4, R, D), BF),
        pltpu.SemaphoreType.DMA((4, NG)), pltpu.SemaphoreType.DMA((4,)),
        pltpu.SemaphoreType.DMA((4,)), pltpu.SemaphoreType.DMA((2, NG)),
    ]
    return pl.pallas_call(
        _kernel,
        out_shape=jax.ShapeDtypeStruct((1, S, 2 * D), BF),
        in_specs=[anyspec, anyspec, anyspec, vm, anyspec, vm, anyspec, anyspec, anyspec, vm, vm, vm],
        out_specs=anyspec,
        scratch_shapes=scratch,
        compiler_params=pltpu.CompilerParams(vmem_limit_bytes=110 * 2 ** 20),
    )(A_q, A_k, A_v, A_shift_k, A_ssm_k, A_ssm_D.reshape(1, D), B_x, B_wqkv, B_wo, _F, _G, _I)
```

```python
import numpy as np
import ml_dtypes
import jax
import jax.numpy as jnp
import jax.experimental.pallas as pl
import jax.experimental.pallas.tpu as pltpu

S, D, C, NCH, NG = 2048, 1024, 128, 16, 8
R = 512
BF, F32, U32 = jnp.bfloat16, jnp.float32, jnp.uint32


def _dft_consts():
    fs = np.concatenate([np.arange(0, 128, 2), np.arange(1, 128, 2)]).reshape(16, 8)
    w = 2 * np.pi * (fs + 0.5) / 256.0
    t = np.arange(128)
    ang = w[:, :, None] * t[None, None, :]
    F = np.concatenate([np.cos(ang), -np.sin(ang)], axis=1).reshape(256, 128)
    G = (F / 128.0).T
    I = np.eye(128)
    b = ml_dtypes.bfloat16
    return F.astype(b), np.ascontiguousarray(G).astype(b), I.astype(b)


_F, _G, _I = _dft_consts()


class P:
    def __init__(self, ref):
        self.r = ref

    def get(self, r0, n, c0, m):
        return pltpu.bitcast(self.r[r0 // 2:(r0 + n) // 2, c0:c0 + m], BF)

    def set(self, r0, c0, val):
        n, m = val.shape
        self.r[r0 // 2:(r0 + n) // 2, c0:c0 + m] = pltpu.bitcast(val, U32)


def _nn(a, b):
    return jnp.dot(a, b, preferred_element_type=F32)


def _nt(a, b):
    return jax.lax.dot_general(a, b, (((1,), (1,)), ((), ())), preferred_element_type=F32)


def _phi(t):
    return jnp.where(t > 0, t + 1.0, jnp.exp(t)) + 1e-6


def _merge(streams):
    streams = [s for s in streams if s]
    tot = [float(sum(c for _, c in s)) for s in streams]
    pos = [0] * len(streams)
    done = [0.0] * len(streams)
    while True:
        best = None
        for i, s in enumerate(streams):
            if pos[i] < len(s):
                key = (done[i] + 0.5 * s[pos[i]][1]) / tot[i]
                if best is None or key < best[0]:
                    best = (key, i)
        if best is None:
            return
        i = best[1]
        th, c = streams[i][pos[i]]
        th()
        done[i] += c
        pos[i] += 1


def _kernel(q_h, k_h, v_h, sh_ref, sk_h, sd_ref, x_h, wqkv_h, wo_h, F_ref, G_ref, I_ref, o_h,
            q_s, k_s, v_s, sk_s, x_s, w_s, wo_s, xp, wkT, wqp, Fp, Gp, par, kf, kvp, Xs, Ks, Yp,
            pkT, Gacc, zacc, Zp, Mp, pqp, op, oA, oB, sA, sB, sW, sO):
    Fp, Gp, wkT, wqp, kvp, Yp, pkT, Zp, Mp, pqp, op = map(
        P, (Fp, Gp, wkT, wqp, kvp, Yp, pkT, Zp, Mp, pqp, op))

    def a_copies(g):
        return [pltpu.make_async_copy(k_h.at[0, :, pl.ds(g * 128, 128)], k_s.at[g], sA.at[0, g]),
                pltpu.make_async_copy(v_h.at[0, :, pl.ds(g * 128, 128)], v_s.at[g], sA.at[1, g]),
                pltpu.make_async_copy(sk_h.at[pl.ds(g * 128, 128), :], sk_s.at[g], sA.at[2, g]),
                pltpu.make_async_copy(q_h.at[0, :, pl.ds(g * 128, 128)], q_s.at[g], sA.at[3, g])]

    def x_copy(i):
        return pltpu.make_async_copy(x_h.at[0, pl.ds(i * R, R), :], x_s.at[i], sB.at[i])

    def w_copy(j):
        return pltpu.make_async_copy(wqkv_h.at[:, pl.ds(j * D, D)], w_s.at[j], sW.at[j])

    wo_copy = pltpu.make_async_copy(wo_h, wo_s, sW.at[3])

    def oa_copy(g):
        return pltpu.make_async_copy(oA.at[g], o_h.at[0, :, pl.ds(g * 128, 128)], sO.at[0, g])

    def ob_copy(i):
        return pltpu.make_async_copy(oB.at[i], o_h.at[0, pl.ds(i * R, R), pl.ds(D, D)], sO.at[1, i])

    w_copy(1).start()
    x_copy(0).start()
    for c in a_copies(0):
        c.start()
    for i in range(1, 4):
        x_copy(i).start()
        for c in a_copies(i):
            c.start()
    w_copy(2).start()
    wo_copy.start()
    w_copy(0).start()
    for g in range(4, NG):
        for c in a_copies(g):
            c.start()

    Fp.set(0, 0, F_ref[...])
    Gp.set(0, 0, G_ref[...])
    shT = sh_ref[...].astype(F32).T
    sd = sd_ref[...].astype(F32)
    for g in range(NG):
        par[g, 0:4, :] = shT[:, g * 128:(g + 1) * 128]
        par[g, 4:5, :] = sd[:, g * 128:(g + 1) * 128]
    kf[0:8, :] = jnp.zeros((8, 128), F32)
    zacc[...] = jnp.zeros(zacc.shape, F32)
    Gacc[...] = jnp.zeros(Gacc.shape, F32)
    w_copy(1).wait()
    eye = I_ref[...]
    for a in range(8):
        for b in range(8):
            t = _nt(eye, w_s[1, a * 128:(a + 1) * 128, b * 128:(b + 1) * 128])
            wkT.set(b * 128, a * 128, t.astype(BF))

    def a_shift(g):
        out = []
        for r in range(0, S, 128):
            def th(r=r):
                kf[8 + r:8 + r + 128, :] = k_s[g, r:r + 128, :].astype(F32)
            out.append((th, 16))
        for r in range(0, S, 32):
            def th(r=r):
                acc = kf[8 + r:8 + r + 32, :] * par[g, 0:1, :]
                for i in range(1, 4):
                    acc = acc + kf[8 + r - i:8 + r - i + 32, :] * par[g, i:i + 1, :]
                kvp.set(r, 0, (acc * v_s[g, r:r + 32, :].astype(F32)).astype(BF))
            out.append((th, 40))
        return out

    def a_dft(g):
        out = []
        for n in range(NCH):
            def th(n=n):
                Ks[n * 256:(n + 1) * 256, :] = _nt(Fp.get(0, 256, 0, 128), sk_s[g, :, n * 128:(n + 1) * 128])
            out.append((th, 64))
        for n in range(NCH):
            def th(n=n):
                Xs[n * 256:(n + 1) * 256, :] = _nn(Fp.get(0, 256, 0, 128), kvp.get(n * 128, 128, 0, 128))
            out.append((th, 64))
        return out

    def a_conv():
        out = []
        for fg in range(16):
            def ld(ref, n, p, fg=fg):
                o = n * 256 + 16 * fg + 8 * p
                return ref[o:o + 8, :]

            def thk(fg=fg, ld=ld):
                for m in range(NCH - 1, 0, -1):
                    kr, ki = ld(Ks, m, 0), ld(Ks, m, 1)
                    pr, pi = ld(Ks, m - 1, 0), ld(Ks, m - 1, 1)
                    o = m * 256 + 16 * fg
                    if fg < 8:
                        Ks[o:o + 8, :] = kr - pi
                        Ks[o + 8:o + 16, :] = ki + pr
                    else:
                        Ks[o:o + 8, :] = kr + pi
                        Ks[o + 8:o + 16, :] = ki - pr
            out.append((thk, 30))
            for n in range(NCH):
                def th(n=n, fg=fg, ld=ld):
                    ar = ai = None
                    for m in range(n + 1):
                        kr, ki = ld(Ks, m, 0), ld(Ks, m, 1)
                        xr, xi = ld(Xs, n - m, 0), ld(Xs, n - m, 1)
                        tr = kr * xr - ki * xi
                        ti = kr * xi + ki * xr
                        ar = tr if ar is None else ar + tr
                        ai = ti if ai is None else ai + ti
                    Yp.set(n * 256 + 16 * fg, 0, jnp.concatenate([ar, ai], axis=0).astype(BF))
                out.append((th, 8 * (n + 1)))
        return out

    def a_inv(g):
        out = []
        for n in range(NCH):
            def th(n=n):
                y = _nn(Gp.get(0, 128, 0, 256), Yp.get(n * 256, 256, 0, 128))
                kv = kvp.get(n * 128, 128, 0, 128).astype(F32)
                y = y + kv * par[g, 4:5, :]
                oA[g, n * 128:(n + 1) * 128, :] = (q_s[g, n * 128:(n + 1) * 128, :].astype(F32) * y).astype(BF)
            out.append((th, 64))
        return out

    def run_step(g, b):
        n = len(b)
        n1 = n // 8

        @pl.when(g > 0)
        def _():
            _merge([a_inv(g - 1)])
            oa_copy(g - 1).start()

        for c in a_copies(g):
            c.wait()
        _merge([b[:n1], a_shift(g)])

        @pl.when(g >= 0)
        def _():
            _merge([a_dft(g)])

        _merge([b[n1:], a_conv()])

    def b1(i):
        X = P(xp.at[i])

        def kproj(c):
            out = []
            for t in range(R // 128):
                st = {}
                for kh in range(2):
                    def th(t=t, kh=kh, st=st):
                        r = _nt(wkT.get(c * 64, 64, kh * 512, 512), X.get(t * 128, 128, kh * 512, 512))
                        if kh == 0:
                            st["a"] = r
                            return
                        p = _phi(r + st["a"])
                        zacc[c * 64:(c + 1) * 64, :] += p
                        pkT.set(c * 64, t * 128, p.astype(BF))
                    out.append((th, 64))
            return out

        def gup(c):
            out = []
            for h in range(8):
                def th(h=h):
                    Gacc[c * 64:(c + 1) * 64, h * 128:(h + 1) * 128] += _nn(
                        pkT.get(c * 64, 64, 0, R), X.get(0, R, h * 128, 128))
                out.append((th, 64))
            return out

        seq = kproj(0)
        for c in range(1, 16):
            seq += kproj(c) + gup(c - 1)
        return seq + gup(15)

    def step1(i, carry):
        x_copy(i).wait()
        for r in range(0, R, 64):
            P(xp.at[i]).set(r, 0, x_s[i, r:r + 64, :])
        run_step(i, b1(i))
        return carry

    jax.lax.fori_loop(0, 4, step1, 0)

    w_copy(2).wait()
    wo_copy.wait()
    w_copy(0).wait()
    for r in range(0, D, 64):
        wqp.set(r, 0, w_s[0, r:r + 64, :])
    ri = jax.lax.broadcasted_iota(jnp.int32, (128, 128), 0) // 32
    ci = jax.lax.broadcasted_iota(jnp.int32, (128, 128), 1) // 32
    mask = ri == ci
    kvs = []
    for g in range(NG):
        z = jnp.sum(zacc[g * 128:(g + 1) * 128, :], axis=1, keepdims=True)
        Zp.set(g * 128, 0, jnp.where(mask, z, 0.0).astype(BF))
        kv = _nn(Gacc[g * 128:(g + 1) * 128, :].astype(BF), w_s[2, :, g * 128:(g + 1) * 128])
        kvs.append(jnp.where(mask, kv, 0.0).astype(BF))
    for g in range(NG):
        for h in range(2):
            Mp.set(g * 128, h * 512, _nn(kvs[g], wo_s[g * 128:(g + 1) * 128, h * 512:(h + 1) * 512]).astype(BF))

    def b2(i):
        X = P(xp.at[i])

        def qproj(t):
            out = []
            for h in range(8):
                st = {}
                for kh in range(2):
                    def th(h=h, kh=kh, st=st):
                        r = _nn(X.get(t * 64, 64, kh * 512, 512), wqp.get(kh * 512, 512, h * 128, 128))
                        if kh == 0:
                            st["a"] = r
                            return
                        pqp.set((t % 2) * 64, h * 128, _phi(r + st["a"]).astype(BF))
                    out.append((th, 64))
            return out

        def den(t):
            out = []
            for hh in range(2):
                def th(hh=hh):
                    for h in range(hh * 4, hh * 4 + 4):
                        pq = pqp.get((t % 2) * 64, 64, h * 128, 128)
                        d = _nn(pq, Zp.get(h * 128, 128, 0, 128)) + 1e-6
                        op.set((t % 2) * 64, h * 128, (pq.astype(F32) / d).astype(BF))
                out.append((th, 64))
            return out

        def oproj(t):
            out = []
            for h in range(8):
                st = {}
                for kh in range(2):
                    def th(h=h, kh=kh, st=st):
                        r = _nn(op.get((t % 2) * 64, 64, kh * 512, 512), Mp.get(kh * 512, 512, h * 128, 128))
                        if kh == 0:
                            st["a"] = r
                            return
                        oB[i, t * 64:(t + 1) * 64, h * 128:(h + 1) * 128] = (r + st["a"]).astype(BF)
                    out.append((th, 64))
            return out

        nt = R // 64
        seq = qproj(0)
        for t in range(nt):
            if t + 1 < nt:
                nx = qproj(t + 1)
                seq += nx[:2] + den(t) + nx[2:]
            else:
                seq += den(t)
            seq += oproj(t)
        return seq

    def step2(i, carry):
        run_step(i + 4, b2(i))
        ob_copy(i).start()
        return carry

    jax.lax.fori_loop(0, 4, step2, 0)

    _merge([a_inv(NG - 1)])
    oa_copy(NG - 1).start()
    for g in range(NG):
        oa_copy(g).wait()
    for i in range(4):
        ob_copy(i).wait()


@jax.jit
def pallas_concat_heads__ssm_conv_h3__linear_attn_block__prompt_kernel(
    A_q, A_k, A_v, A_shift_k, A_ssm_k, A_ssm_D, B_x, B_wqkv, B_wo,
):
    anyspec = pl.BlockSpec(memory_space=pl.ANY)
    vm = pl.BlockSpec(memory_space=pltpu.VMEM)
    V = pltpu.VMEM
    scratch = [
        V((NG, S, 128), BF), V((NG, S, 128), BF), V((NG, S, 128), BF), V((NG, 128, S), BF),
        V((4, R, D), BF), V((3, D, D), BF), V((D, D), BF),
        V((4, R // 2, D), U32), V((D // 2, D), U32), V((D // 2, D), U32),
        V((128, 128), U32), V((64, 256), U32), V((NG, 8, 128), F32), V((S + 8, 128), F32),
        V((S // 2, 128), U32), V((2 * S, 128), F32), V((2 * S, 128), F32), V((S, 128), U32),
        V((D // 2, R), U32), V((D, D), F32), V((D, 128), F32), V((D // 2, 128), U32),
        V((D // 2, D), U32), V((64, D), U32), V((64, D), U32),
        V((NG, S, 128), BF), V((4, R, D), BF),
        pltpu.SemaphoreType.DMA((4, NG)), pltpu.SemaphoreType.DMA((4,)),
        pltpu.SemaphoreType.DMA((4,)), pltpu.SemaphoreType.DMA((2, NG)),
    ]
    return pl.pallas_call(
        _kernel,
        out_shape=jax.ShapeDtypeStruct((1, S, 2 * D), BF),
        in_specs=[anyspec, anyspec, anyspec, vm, anyspec, vm, anyspec, anyspec, anyspec, vm, vm, vm],
        out_specs=anyspec,
        scratch_shapes=scratch,
        compiler_params=pltpu.CompilerParams(vmem_limit_bytes=110 * 2 ** 20),
    )(A_q, A_k, A_v, A_shift_k, A_ssm_k, A_ssm_D.reshape(1, D), B_x, B_wqkv, B_wo, _F, _G, _I)
```
